```python
import jax
import jax.numpy as jnp

def _softmax(x, axis=-1):
    return jax.nn.softmax(x, axis=axis)
def _gelu(x):
    return jax.nn.gelu(x, approximate=True)
def _silu(x):
    return jax.nn.silu(x)
def _sigmoid(x):
    return jax.nn.sigmoid(x)
def _layernorm(x, axis=-1, eps=1e-5):
    m = jnp.mean(x, axis=axis, keepdims=True)
    v = jnp.var(x, axis=axis, keepdims=True)
    return (x - m) / jnp.sqrt(v + eps)
def _scatter_add(tgt, idx, src, axis=0):
    return tgt.at[idx].add(src)
def _segment_sum(src, seg, n):
    return jax.ops.segment_sum(src, seg, n)
class _Rng:
    def __init__(self, key):
        self._k = key
    def _next(self):
        self._k, sub = jax.random.split(self._k)
        return sub
    def normal(self, shape):
        return jax.random.normal(self._next(), shape, dtype=jnp.bfloat16)
    def randint(self, lo, hi, shape):
        return jax.random.randint(self._next(), shape, lo, hi, dtype=jnp.int32)
    def uniform(self, shape, lo=0.0, hi=1.0):
        return jax.random.uniform(self._next(), shape, jnp.bfloat16, lo, hi)
    def permutation(self, n):
        return jax.random.permutation(self._next(), n)


kernel_name = 'standalone__standard_2d_1d_3d_conv__vision'

def setup_inputs():
    _rng = _Rng(jax.random.key(int.from_bytes(__import__("os").urandom(4), "little")))
    _w = (lambda a: (lambda t: t.astype(jnp.bfloat16) if jnp.issubdtype(t.dtype, jnp.floating) else t)(jnp.asarray(a)))
    H = W = 384
    C = 384
    K = 1
    return {
        "x": _w((lambda *s: _rng.normal(s) * 0.05)(1, H, W, C)),
        "w": _w((lambda *s: _rng.normal(s) * 0.05)(K, K, C, C)),
        "b": _w((lambda *s: _rng.normal(s) * 0.05)(C)),
    }

def reference(x, w, b):
    B, H, W, Cin = x.shape
    K = w.shape[0]
    pl = (K - 1) // 2
    pr = K // 2
    xp = jnp.pad(x, ((0, 0), (pl, pr), (pl, pr), (0, 0)))
    out = sum(
        jnp.einsum('bhwc,cd->bhwd', xp[:, i:i+H, j:j+W, :], w[i, j])
        for i in range(K) for j in range(K)
    )
    return out + b[None, None, None, :]
```

```python
import jax
import jax.numpy as jnp
import jax.experimental.pallas as pl
import jax.experimental.pallas.tpu as pltpu

_TM = 1536
_READ_ROWS = 6144
_READ_TAIL = 512
_PIECE = 32
_STREAMS = 6
_STREAM_ROWS = 4096
_READ_STEPS = 56
_FIRST_WRITES = 16
_WRITES_PER_STEP = 13


@jax.jit
def pallas_standalone__standard_2d_1d_3d_conv__vision_kernel(
    x: jax.Array,
    w: jax.Array,
    b: jax.Array,
):
    B, H, W, C = x.shape
    assert w.shape == (1, 1, C, C), "only the 1x1 convolution is implemented"
    M = B * H * W
    group_rows = _STREAMS * _STREAM_ROWS
    assert M % group_rows == 0 and M % _READ_ROWS == 0 and _READ_ROWS % _TM == 0
    n_steps = M // _TM
    steps_per_read = _READ_ROWS // _TM
    writes_per_group = _STREAM_ROWS // _PIECE
    n_writes = (M // group_rows) * writes_per_group
    read_bounds = list(range(0, M, _READ_ROWS)) + [M - _READ_TAIL, M]
    n_reads = len(read_bounds) - 1
    for i in range(_READ_STEPS, n_steps):
        last = _FIRST_WRITES + (i - _READ_STEPS + 1) * _WRITES_PER_STEP - 1
        assert last < n_writes
        assert (last // writes_per_group + 1) * group_rows <= i * _TM

    def kernel(x_hbm, w_hbm, b_hbm, o_hbm, buf, w_vmem, b_vmem,
               read_sems, write_sem, param_sems):
        def read(k):
            rows = pl.ds(read_bounds[k], read_bounds[k + 1] - read_bounds[k])
            return pltpu.make_async_copy(
                x_hbm.at[rows], buf.at[rows], read_sems.at[k])

        w_copy = pltpu.make_async_copy(w_hbm, w_vmem, param_sems.at[0])
        b_copy = pltpu.make_async_copy(b_hbm, b_vmem, param_sems.at[1])
        w_copy.start()
        b_copy.start()
        for k in range(n_reads):
            read(k).start(priority=1)
        w_copy.wait()
        b_copy.wait()
        bias = b_vmem[...].astype(jnp.float32).reshape(1, C)

        src = buf.reshape(M // _STREAM_ROWS, _STREAM_ROWS, C)
        dst = o_hbm.reshape(M // _STREAM_ROWS, _STREAM_ROWS, C)

        def start_write(q):
            streams = pl.ds((q // writes_per_group) * _STREAMS, _STREAMS)
            rows = pl.ds(
                pl.multiple_of((q % writes_per_group) * _PIECE, _PIECE), _PIECE)
            pltpu.make_async_copy(
                src.at[streams, rows], dst.at[streams, rows], write_sem.at[0]
            ).start()

        def compute(i):
            rows = pl.ds(pl.multiple_of(i * _TM, _TM), _TM)
            acc = jnp.dot(buf[rows, :], w_vmem[...],
                          preferred_element_type=jnp.float32)
            buf[rows, :] = (acc + bias).astype(buf.dtype)

        def read_phase_step(i, carry):
            @pl.when(i % steps_per_read == 0)
            def _():
                k = i // steps_per_read
                rows = pl.ds(pl.multiple_of(k * _READ_ROWS, _READ_ROWS),
                             _READ_ROWS)
                pltpu.make_async_copy(
                    x_hbm.at[rows], buf.at[rows], read_sems.at[k]).wait()

            compute(i)
            return carry

        jax.lax.fori_loop(0, _READ_STEPS, read_phase_step, 0)

        for k in range(pl.cdiv(_READ_STEPS, steps_per_read), n_reads - 1):
            read(k).wait()
        for q in range(_FIRST_WRITES):
            start_write(q)
        read(n_reads - 1).wait()

        def write_phase_step(i, carry):
            q0 = _FIRST_WRITES + (i - _READ_STEPS) * _WRITES_PER_STEP
            for u in range(_WRITES_PER_STEP):
                start_write(q0 + u)
            compute(i)
            return carry

        jax.lax.fori_loop(_READ_STEPS, n_steps, write_phase_step, 0)

        def drain_step(q, carry):
            start_write(q)
            return carry

        jax.lax.fori_loop(
            _FIRST_WRITES + (n_steps - _READ_STEPS) * _WRITES_PER_STEP,
            n_writes, drain_step, 0)
        pltpu.make_async_copy(buf, o_hbm, write_sem.at[0]).wait()

    out = pl.pallas_call(
        kernel,
        in_specs=[pl.BlockSpec(memory_space=pltpu.HBM)] * 3,
        out_specs=pl.BlockSpec(memory_space=pltpu.HBM),
        out_shape=jax.ShapeDtypeStruct((M, C), x.dtype),
        scratch_shapes=[
            pltpu.VMEM((M, C), x.dtype),
            pltpu.VMEM((C, C), w.dtype),
            pltpu.VMEM((C,), b.dtype),
            pltpu.SemaphoreType.DMA((n_reads,)),
            pltpu.SemaphoreType.DMA((1,)),
            pltpu.SemaphoreType.DMA((2,)),
        ],
        compiler_params=pltpu.CompilerParams(
            vmem_limit_bytes=124 * 2**20,
            disable_bounds_checks=True,
        ),
    )(x.reshape(M, C), w.reshape(C, C), b)
    return out.reshape(B, H, W, C)
```

```python
import jax
import jax.numpy as jnp
import jax.experimental.pallas as pl
import jax.experimental.pallas.tpu as pltpu

_LANES = 128
_SUBLANES = 8
_BLOCK = 128
_PARTS = 2
_BUFFERS = 4
_STEP_STREAMS = 3

_READ_STREAM_BLOCKS = 8
_READ_PIECE = 128
_REGION_STREAMS = 15
_REGIONS = 7
_LARGE_AHEAD = 6
_LARGE_RATE = (3, 4)
_SMALL_MASK = (1, 1, 0)
_SMALL_DELAY_NS = 120
_READ_STEPS = 52

_WRITE_STREAM_BLOCKS = 32
_WRITE_PIECE = 96
_WRITE_STREAMS = 6
_WRITE_RATE = (13, 16)


def _divmod(i, d):
    if isinstance(i, int):
        return divmod(i, d)
    q = jax.lax.div(i.astype(jnp.uint32), jnp.uint32(d)).astype(jnp.int32)
    return q, i - q * d


@jax.jit
def pallas_standalone__standard_2d_1d_3d_conv__vision_kernel(
    x: jax.Array,
    w: jax.Array,
    b: jax.Array,
):
    B, H, W, C = x.shape
    assert w.shape == (1, 1, C, C), "only the 1x1 convolution is implemented"
    M = B * H * W
    col_tiles = C // _LANES
    block_rows = _BLOCK * col_tiles
    n_blocks = M // _BLOCK
    n_steps = n_blocks // (_STEP_STREAMS * _BUFFERS)

    n_streams = n_blocks // _READ_STREAM_BLOCKS
    stream_tuples = _READ_STREAM_BLOCKS // _BUFFERS
    block_pieces = block_rows // _READ_PIECE
    n_units = _REGIONS * stream_tuples
    unit_steps = _REGION_STREAMS // _STEP_STREAMS
    n_large = n_units * block_pieces
    large_streams = _REGIONS * _REGION_STREAMS
    small_streams = n_streams - large_streams
    large_steps = n_units * unit_steps
    parts = [(s, h, a) for s in range(_STEP_STREAMS) for h in range(_PARTS)
             for a in range(_BUFFERS)]
    small_per_step = sum(
        _SMALL_MASK[q % len(_SMALL_MASK)] for q in range(len(parts))) // _BUFFERS
    small_before = (small_streams * stream_tuples * block_pieces
                    - _READ_STEPS * small_per_step)

    write_tuples = _WRITE_STREAM_BLOCKS // _BUFFERS
    n_write_streams = n_blocks // _WRITE_STREAM_BLOCKS
    n_writes = (n_write_streams // _WRITE_STREAMS) * write_tuples

    def step_position(i):
        if isinstance(i, int):
            select, j = (lambda c, p, q: p if c else q), max(i - large_steps, 0)
        else:
            select, j = jnp.where, jnp.maximum(i - large_steps, 0)
        unit, unit_step = _divmod(i, unit_steps)
        region, region_index = _divmod(unit, stream_tuples)
        group, group_index = _divmod(j, stream_tuples)
        stream = select(
            i < large_steps,
            region * _REGION_STREAMS + unit_step * _STEP_STREAMS,
            large_streams + group * _STEP_STREAMS)
        return stream, select(i < large_steps, region_index, group_index)

    def large_started_before(i):
        return _LARGE_AHEAD + _divmod(i * _LARGE_RATE[0], _LARGE_RATE[1])[0]

    def writes_started_before(i):
        return 2 + _divmod(
            (i - _READ_STEPS) * _WRITE_RATE[0], _WRITE_RATE[1])[0]

    assert C % _LANES == 0 and n_blocks * _BLOCK == M
    assert n_streams * _READ_STREAM_BLOCKS == n_blocks
    assert n_write_streams % _WRITE_STREAMS == 0
    assert _REGION_STREAMS % _STEP_STREAMS == 0
    assert small_streams > 0 and small_streams % _STEP_STREAMS == 0
    assert small_before >= 0 and _READ_STEPS <= large_steps - unit_steps
    assert large_started_before(_READ_STEPS) >= n_large
    for a in range(_BUFFERS):
        assert small_per_step == sum(
            _SMALL_MASK[q % len(_SMALL_MASK)]
            for q, part in enumerate(parts) if part[2] == a)
    done = set()
    for i in range(n_steps):
        if i < _READ_STEPS:
            assert large_started_before(i + 1) >= min(
                n_large, (i // unit_steps + 1) * block_pieces)
        else:
            group = (writes_started_before(i + 1) - 1) // write_tuples
            assert done.issuperset(
                range((group + 1) * _WRITE_STREAMS * _WRITE_STREAM_BLOCKS))
        stream, index = step_position(i)
        done.update(
            (stream + s) * _READ_STREAM_BLOCKS + index * _BUFFERS + a
            for s in range(_STEP_STREAMS) for a in range(_BUFFERS))
    assert len(done) == n_blocks

    def kernel(x_hbm, w_hbm, b_hbm, o_hbm, w_vmem, b_vmem,
               param_sems, large_sems, small_sems, write_sems, *bufs):
        w_copy = pltpu.make_async_copy(w_hbm, w_vmem, param_sems.at[0])
        b_copy = pltpu.make_async_copy(b_hbm, b_vmem, param_sems.at[1])
        w_copy.start()
        b_copy.start()

        x_streams = x_hbm.reshape(
            n_streams, _READ_STREAM_BLOCKS, block_rows, _LANES)
        buf_streams = [
            buf.reshape(n_streams, stream_tuples, block_rows, _LANES)
            for buf in bufs]

        def start_large(m):
            unit, piece = _divmod(m, block_pieces)
            region, index = _divmod(unit, stream_tuples)
            streams = pl.ds(region * _REGION_STREAMS, _REGION_STREAMS)
            start = piece * _READ_PIECE
            if isinstance(m, int):
                last_sem = n_units if m == n_large - 1 else unit
            else:
                start = pl.multiple_of(start, _READ_PIECE)
                last_sem = jnp.where(m == n_large - 1, n_units, unit)
            rows = pl.ds(start, _READ_PIECE)
            for a in range(_BUFFERS):
                sem = last_sem if a == _BUFFERS - 1 else unit
                pltpu.make_async_copy(
                    x_streams.at[streams, index * _BUFFERS + a, rows],
                    buf_streams[a].at[streams, index, rows],
                    large_sems.at[sem],
                ).start(priority=1)

        def wait_large(sem, count):
            shape = (pl.ds(0, _REGION_STREAMS), 0, pl.ds(0, _READ_PIECE))
            for _ in range(count):
                pltpu.make_async_copy(
                    x_streams.at[shape], buf_streams[0].at[shape],
                    large_sems.at[sem]).wait()

        def start_small(t, a):
            piece, stream = _divmod(t, small_streams)
            index, piece = _divmod(piece, block_pieces)
            rows = pl.ds(
                pl.multiple_of(piece * _READ_PIECE, _READ_PIECE), _READ_PIECE)
            pltpu.make_async_copy(
                x_streams.at[large_streams + stream, index * _BUFFERS + a, rows],
                buf_streams[a].at[large_streams + stream, index, rows],
                small_sems.at[a]).start()

        for m in range(_LARGE_AHEAD):
            start_large(m)

        def early_small_reads(t, carry):
            for a in range(_BUFFERS):
                start_small(t, a)
                pl.delay(_SMALL_DELAY_NS)
            return carry

        jax.lax.fori_loop(0, small_before, early_small_reads, 0)
        w_copy.wait()
        b_copy.wait()
        bias = b_vmem[...].astype(jnp.float32).reshape(1, C)

        def multiply(tiles, pixels):
            groups = pixels // _SUBLANES
            tiles = tiles.reshape(groups, col_tiles, _SUBLANES, _LANES)
            lhs = jnp.concatenate(
                [tiles[:, c].reshape(pixels, _LANES) for c in range(col_tiles)],
                axis=1)
            acc = jnp.dot(lhs, w_vmem[...],
                          preferred_element_type=jnp.float32) + bias
            tiles = jnp.concatenate(
                [acc[:, c * _LANES:(c + 1) * _LANES].reshape(
                    groups, 1, _SUBLANES, _LANES) for c in range(col_tiles)],
                axis=1)
            return tiles.reshape(pixels * col_tiles, _LANES).astype(x.dtype)

        def read_phase_step(i, carry):
            m = large_started_before(i)

            @pl.when(jnp.logical_and(m < n_large,
                                     large_started_before(i + 1) > m))
            def _():
                start_large(m)

            unit, unit_step = _divmod(i, unit_steps)

            @pl.when(unit_step == 0)
            def _():
                wait_large(unit, block_pieces * _BUFFERS)

            stream, index = step_position(i)
            pixels = _BLOCK // _PARTS
            started = [0] * _BUFFERS
            for q, (s, h, a) in enumerate(parts):
                rows = pl.ds(h * pixels * col_tiles, pixels * col_tiles)
                buf = buf_streams[a]
                buf[stream + s, index, rows] = multiply(
                    buf[stream + s, index, rows], pixels)
                if _SMALL_MASK[q % len(_SMALL_MASK)]:
                    start_small(
                        small_before + i * small_per_step + started[a], a)
                    started[a] += 1
            return carry

        jax.lax.fori_loop(0, _READ_STEPS, read_phase_step, 0)

        o_streams = o_hbm.reshape(
            n_write_streams, _WRITE_STREAM_BLOCKS, block_rows, _LANES)
        buf_write_streams = [
            buf.reshape(n_write_streams, write_tuples, block_rows, _LANES)
            for buf in bufs]

        def start_writes(t):
            group, index = _divmod(t, write_tuples)
            streams = pl.ds(group * _WRITE_STREAMS, _WRITE_STREAMS)
            for a in range(_BUFFERS):
                for start in range(0, block_rows, _WRITE_PIECE):
                    rows = pl.ds(start, _WRITE_PIECE)
                    pltpu.make_async_copy(
                        buf_write_streams[a].at[streams, index, rows],
                        o_streams.at[streams, index * _BUFFERS + a, rows],
                        write_sems.at[a]).start(priority=1)

        for unit in range(pl.cdiv(_READ_STEPS, unit_steps), n_units):
            wait_large(
                unit, block_pieces * _BUFFERS - (unit == n_units - 1))
        start_writes(0)
        wait_large(n_units, 1)
        for a in range(_BUFFERS):
            region = buf_streams[a].at[pl.ds(large_streams, small_streams)]
            pltpu.make_async_copy(region, region, small_sems.at[a]).wait()
        start_writes(1)

        def write_phase_step(i, carry):
            t = writes_started_before(i)

            @pl.when(writes_started_before(i + 1) > t)
            def _():
                start_writes(t)

            stream, index = step_position(i)
            streams = pl.ds(stream, _STEP_STREAMS)
            for buf in buf_streams:
                buf[streams, index] = multiply(
                    buf[streams, index], _STEP_STREAMS * _BLOCK
                ).reshape(_STEP_STREAMS, block_rows, _LANES)
            return carry

        jax.lax.fori_loop(_READ_STEPS, n_steps, write_phase_step, 0)

        def remaining_writes(t, carry):
            start_writes(t)
            return carry

        jax.lax.fori_loop(
            writes_started_before(n_steps), n_writes, remaining_writes, 0)
        for a in range(_BUFFERS):
            pltpu.make_async_copy(bufs[a], bufs[a], write_sems.at[a]).wait()

    x_tiles = (x.reshape(M // _SUBLANES, _SUBLANES, col_tiles, _LANES)
               .transpose(0, 2, 1, 3).reshape(M * col_tiles, _LANES))
    out_tiles = pl.pallas_call(
        kernel,
        in_specs=[pl.BlockSpec(memory_space=pltpu.HBM)] * 3,
        out_specs=pl.BlockSpec(memory_space=pltpu.HBM),
        out_shape=jax.ShapeDtypeStruct(x_tiles.shape, x.dtype),
        scratch_shapes=[
            pltpu.VMEM((C, C), w.dtype),
            pltpu.VMEM((C,), b.dtype),
            pltpu.SemaphoreType.DMA((2,)),
            pltpu.SemaphoreType.DMA((n_units + 1,)),
            pltpu.SemaphoreType.DMA((_BUFFERS,)),
            pltpu.SemaphoreType.DMA((_BUFFERS,)),
        ] + [pltpu.VMEM((M * col_tiles // _BUFFERS, _LANES), x.dtype)] * _BUFFERS,
        compiler_params=pltpu.CompilerParams(
            vmem_limit_bytes=124 * 2**20,
            disable_bounds_checks=True,
        ),
    )(x_tiles, w.reshape(C, C), b)
    return (out_tiles.reshape(M // _SUBLANES, col_tiles, _SUBLANES, _LANES)
            .transpose(0, 2, 1, 3).reshape(B, H, W, C))
```

```python
import jax
import jax.numpy as jnp
import numpy as np
import jax.experimental.pallas as pl
import jax.experimental.pallas.tpu as pltpu

_LANES = 128
_SUBLANES = 8
_BLOCK = 128
_PARTS = 2
_BUFFERS = 4
_STEP_STREAMS = 3

_READ_STREAM_BLOCKS = 8
_READ_PIECE = 128
_REGION_STREAMS = 15
_REGIONS = 7
_LARGE_AHEAD = 6
_LARGE_RATE = (3, 4)
_READ_STEPS = 52
_SMALL_DELAY_NS = 120
_SMALL_AFTER = (1, 2, 4, 5, 7, 9, 10, 12, 14, 16, 17, 19, 20, 22, 23)

_WRITE_STREAM_BLOCKS = 32
_WRITE_PIECE = 96
_WRITE_STREAMS = 6
_WRITE_RATE = (13, 16)


def _divmod(i, d):
    if isinstance(i, int):
        return divmod(i, d)
    q = jax.lax.div(i.astype(jnp.uint32), np.uint32(d)).astype(jnp.int32)
    return q, i - q * d


@jax.jit
def pallas_standalone__standard_2d_1d_3d_conv__vision_kernel(
    x: jax.Array,
    w: jax.Array,
    b: jax.Array,
):
    B, H, W, C = x.shape
    assert w.shape == (1, 1, C, C), "only the 1x1 convolution is implemented"
    M = B * H * W
    col_tiles = C // _LANES
    block_rows = _BLOCK * col_tiles
    n_blocks = M // _BLOCK
    n_steps = n_blocks // (_STEP_STREAMS * _BUFFERS)

    n_streams = n_blocks // _READ_STREAM_BLOCKS
    stream_tuples = _READ_STREAM_BLOCKS // _BUFFERS
    block_pieces = block_rows // _READ_PIECE
    n_units = _REGIONS * stream_tuples
    unit_steps = _REGION_STREAMS // _STEP_STREAMS
    n_large = n_units * block_pieces
    large_streams = _REGIONS * _REGION_STREAMS
    small_streams = n_streams - large_streams
    large_steps = n_units * unit_steps
    parts = [(s, h, a) for s in range(_STEP_STREAMS) for h in range(_PARTS)
             for a in range(_BUFFERS)]
    small_buffers = [_BUFFERS - 1] + [parts[q][2] for q in _SMALL_AFTER]
    small_per_step = len(small_buffers) // _BUFFERS
    small_before = (small_streams * stream_tuples * block_pieces
                    - _READ_STEPS * small_per_step)

    write_tuples = _WRITE_STREAM_BLOCKS // _BUFFERS
    n_write_streams = n_blocks // _WRITE_STREAM_BLOCKS
    n_writes = (n_write_streams // _WRITE_STREAMS) * write_tuples

    def step_position(i):
        if isinstance(i, int):
            select, j = (lambda c, p, q: p if c else q), max(i - large_steps, 0)
        else:
            select, j = jnp.where, jnp.maximum(i - large_steps, 0)
        unit, unit_step = _divmod(i, unit_steps)
        region, region_index = _divmod(unit, stream_tuples)
        group, group_index = _divmod(j, stream_tuples)
        stream = select(
            i < large_steps,
            region * _REGION_STREAMS + unit_step * _STEP_STREAMS,
            large_streams + group * _STEP_STREAMS)
        return stream, select(i < large_steps, region_index, group_index)

    def large_started_before(i):
        return _LARGE_AHEAD + _divmod(i * _LARGE_RATE[0], _LARGE_RATE[1])[0]

    def writes_started_before(i):
        return 2 + _divmod(
            (i - _READ_STEPS) * _WRITE_RATE[0], _WRITE_RATE[1])[0]

    assert C % _LANES == 0 and n_blocks * _BLOCK == M
    assert n_streams * _READ_STREAM_BLOCKS == n_blocks
    assert n_write_streams % _WRITE_STREAMS == 0
    assert _REGION_STREAMS % _STEP_STREAMS == 0
    assert small_streams > 0 and small_streams % _STEP_STREAMS == 0
    assert small_before >= 0 and _READ_STEPS <= large_steps - unit_steps
    assert large_started_before(_READ_STEPS) >= n_large
    assert all(small_buffers.count(a) == small_per_step
               for a in range(_BUFFERS))
    done = set()
    for i in range(n_steps):
        if i < _READ_STEPS:
            assert large_started_before(i + 1) >= min(
                n_large, (i // unit_steps + 1) * block_pieces)
        else:
            group = (writes_started_before(i + 1) - 1) // write_tuples
            assert done.issuperset(
                range((group + 1) * _WRITE_STREAMS * _WRITE_STREAM_BLOCKS))
        stream, index = step_position(i)
        done.update(
            (stream + s) * _READ_STREAM_BLOCKS + index * _BUFFERS + a
            for s in range(_STEP_STREAMS) for a in range(_BUFFERS))
    assert len(done) == n_blocks

    def kernel(x_hbm, w_hbm, b_hbm, o_hbm, w_vmem, b_vmem,
               param_sems, large_sems, small_sems, write_sems, *bufs):
        w_copy = pltpu.make_async_copy(w_hbm, w_vmem, param_sems.at[0])
        b_copy = pltpu.make_async_copy(b_hbm, b_vmem, param_sems.at[1])
        w_copy.start()
        b_copy.start()

        x_streams = x_hbm.reshape(
            n_streams, _READ_STREAM_BLOCKS, block_rows, _LANES)
        buf_streams = [
            buf.reshape(n_streams, stream_tuples, block_rows, _LANES)
            for buf in bufs]

        def piece_rows(piece):
            start = piece * _READ_PIECE
            if not isinstance(start, int):
                start = pl.multiple_of(start, _READ_PIECE)
            return pl.ds(start, _READ_PIECE)

        def large_read(unit, piece, a):
            region, index = _divmod(unit, stream_tuples)
            streams = pl.ds(region * _REGION_STREAMS, _REGION_STREAMS)
            sem = unit
            if a == _BUFFERS - 1:
                last = unit * block_pieces + piece == n_large - 1
                if isinstance(last, bool):
                    sem = n_units if last else unit
                else:
                    sem = jnp.where(last, n_units, unit)
            return pltpu.make_async_copy(
                x_streams.at[streams, index * _BUFFERS + a, piece_rows(piece)],
                buf_streams[a].at[streams, index, piece_rows(piece)],
                large_sems.at[sem])

        def start_large(m):
            unit, piece = _divmod(m, block_pieces)
            for a in range(_BUFFERS):
                large_read(unit, piece, a).start(priority=1)

        unit_reads = [(piece, a) for piece in range(block_pieces)
                      for a in range(_BUFFERS)]

        def start_small(t, a):
            piece, stream = _divmod(t, small_streams)
            index, piece = _divmod(piece, block_pieces)
            stream += large_streams
            pltpu.make_async_copy(
                x_streams.at[stream, index * _BUFFERS + a, piece_rows(piece)],
                buf_streams[a].at[stream, index, piece_rows(piece)],
                small_sems.at[a]).start()

        for m in range(_LARGE_AHEAD):
            start_large(m)

        def early_small_reads(t, carry):
            for a in range(_BUFFERS):
                start_small(t, a)
                pl.delay(_SMALL_DELAY_NS)
            return carry

        jax.lax.fori_loop(0, small_before, early_small_reads, 0)
        w_copy.wait()
        b_copy.wait()
        bias = b_vmem[...].astype(jnp.float32).reshape(1, C)

        def multiply(tiles, pixels):
            groups = pixels // _SUBLANES
            tiles = tiles.reshape(groups, col_tiles, _SUBLANES, _LANES)
            lhs = jnp.concatenate(
                [tiles[:, c].reshape(pixels, _LANES) for c in range(col_tiles)],
                axis=1)
            acc = jnp.dot(lhs, w_vmem[...],
                          preferred_element_type=jnp.float32) + bias
            tiles = jnp.concatenate(
                [acc[:, c * _LANES:(c + 1) * _LANES].reshape(
                    groups, 1, _SUBLANES, _LANES) for c in range(col_tiles)],
                axis=1)
            return tiles.reshape(pixels * col_tiles, _LANES).astype(x.dtype)

        def read_phase_step(i, carry):
            m = large_started_before(i)

            @pl.when(jnp.logical_and(m < n_large,
                                     large_started_before(i + 1) > m))
            def _():
                start_large(m)

            unit, unit_step = _divmod(i, unit_steps)

            @pl.when(unit_step == 0)
            def _():
                for piece, a in unit_reads:
                    large_read(unit, piece, a).wait()

            stream, index = step_position(i)
            pixels = _BLOCK // _PARTS
            started = [0] * _BUFFERS

            def next_small(a):
                start_small(small_before + i * small_per_step + started[a], a)
                started[a] += 1

            next_small(small_buffers[0])
            for q, (s, h, a) in enumerate(parts):
                rows = pl.ds(h * pixels * col_tiles, pixels * col_tiles)
                buf = buf_streams[a]
                buf[stream + s, index, rows] = multiply(
                    buf[stream + s, index, rows], pixels)
                if q in _SMALL_AFTER:
                    next_small(a)
            return carry

        jax.lax.fori_loop(0, _READ_STEPS, read_phase_step, 0)

        o_streams = o_hbm.reshape(
            n_write_streams, _WRITE_STREAM_BLOCKS, block_rows, _LANES)
        buf_write_streams = [
            buf.reshape(n_write_streams, write_tuples, block_rows, _LANES)
            for buf in bufs]

        def start_writes(t):
            group, index = _divmod(t, write_tuples)
            streams = pl.ds(group * _WRITE_STREAMS, _WRITE_STREAMS)
            for a in range(_BUFFERS):
                for start in range(0, block_rows, _WRITE_PIECE):
                    rows = pl.ds(start, _WRITE_PIECE)
                    pltpu.make_async_copy(
                        buf_write_streams[a].at[streams, index, rows],
                        o_streams.at[streams, index * _BUFFERS + a, rows],
                        write_sems.at[a]).start(priority=1)

        for unit in range(pl.cdiv(_READ_STEPS, unit_steps), n_units):
            for piece, a in unit_reads:
                if (unit, (piece, a)) == (n_units - 1, unit_reads[-1]):
                    start_writes(0)
                large_read(unit, piece, a).wait()
        for a in range(_BUFFERS):
            region = buf_streams[a].at[pl.ds(large_streams, small_streams)]
            pltpu.make_async_copy(region, region, small_sems.at[a]).wait()
        start_writes(1)

        def write_phase_step(i, carry):
            t = writes_started_before(i)

            @pl.when(writes_started_before(i + 1) > t)
            def _():
                start_writes(t)

            stream, index = step_position(i)
            streams = pl.ds(stream, _STEP_STREAMS)
            for buf in buf_streams:
                buf[streams, index] = multiply(
                    buf[streams, index], _STEP_STREAMS * _BLOCK
                ).reshape(_STEP_STREAMS, block_rows, _LANES)
            return carry

        jax.lax.fori_loop(_READ_STEPS, n_steps, write_phase_step, 0)

        def remaining_writes(t, carry):
            start_writes(t)
            return carry

        jax.lax.fori_loop(
            writes_started_before(n_steps), n_writes, remaining_writes, 0)
        for a in range(_BUFFERS):
            pltpu.make_async_copy(bufs[a], bufs[a], write_sems.at[a]).wait()

    x_tiles = (x.reshape(M // _SUBLANES, _SUBLANES, col_tiles, _LANES)
               .transpose(0, 2, 1, 3).reshape(M * col_tiles, _LANES))
    out_tiles = pl.pallas_call(
        kernel,
        in_specs=[pl.BlockSpec(memory_space=pltpu.HBM)] * 3,
        out_specs=pl.BlockSpec(memory_space=pltpu.HBM),
        out_shape=jax.ShapeDtypeStruct(x_tiles.shape, x.dtype),
        scratch_shapes=[
            pltpu.VMEM((C, C), w.dtype),
            pltpu.VMEM((C,), b.dtype),
            pltpu.SemaphoreType.DMA((2,)),
            pltpu.SemaphoreType.DMA((n_units + 1,)),
            pltpu.SemaphoreType.DMA((_BUFFERS,)),
            pltpu.SemaphoreType.DMA((_BUFFERS,)),
        ] + [pltpu.VMEM((M * col_tiles // _BUFFERS, _LANES), x.dtype)] * _BUFFERS,
        compiler_params=pltpu.CompilerParams(
            vmem_limit_bytes=124 * 2**20,
            disable_bounds_checks=True,
        ),
    )(x_tiles, w.reshape(C, C), b)
    return (out_tiles.reshape(M // _SUBLANES, col_tiles, _SUBLANES, _LANES)
            .transpose(0, 2, 1, 3).reshape(B, H, W, C))
```

```python
import jax
import jax.numpy as jnp
import numpy as np
import jax.experimental.pallas as pl
import jax.experimental.pallas.tpu as pltpu

_LANES = 128
_SUBLANES = 8
_BLOCK = 128
_BUFFERS = 4
_STREAMS = 6
_STREAM_BLOCKS = 8

_PART = 144
_STEP_PARTS = 4

_READ_PIECE = 128
_READ_ORDER = (0, 3, 1, 4, 2, 5)
_READ_PRIORITIES = (0, 1, 1, 1)
_UNIT_BLOCKS = 4
_EXTRA_ROUNDS = 4

_WRITE_PIECE = 96
_WRITE_BLOCKS = 4
_FIRST_WRITES = 3
_WRITE_RATE = (19, 16)


def _divmod(i, d):
    if isinstance(i, int):
        return divmod(i, d)
    q = jax.lax.div(i.astype(jnp.uint32), np.uint32(d)).astype(jnp.int32)
    return q, i - q * d


def _rows(index, size):
    start = index * size
    if not isinstance(start, int):
        start = pl.multiple_of(start, size)
    return pl.ds(start, size)


@jax.jit
def pallas_standalone__standard_2d_1d_3d_conv__vision_kernel(
    x: jax.Array,
    w: jax.Array,
    b: jax.Array,
):
    B, H, W, C = x.shape
    assert w.shape == (1, 1, C, C), "only the 1x1 convolution is implemented"
    M = B * H * W
    col_tiles = C // _LANES
    block_rows = _BLOCK * col_tiles
    n_regions = M // (_BLOCK * _STREAM_BLOCKS * _BUFFERS * _STREAMS)
    step_pixels = _PART * _STEP_PARTS
    n_steps = M // (_BUFFERS * step_pixels)

    block_pieces = block_rows // _READ_PIECE
    unit_rounds = _UNIT_BLOCKS * block_pieces
    unit_pixels = _UNIT_BLOCKS * _STREAMS * _BLOCK
    n_units = n_regions * _STREAM_BLOCKS // _UNIT_BLOCKS
    early_rounds = unit_rounds + _EXTRA_ROUNDS
    read_steps = (n_units * unit_rounds - early_rounds) // _STEP_PARTS

    stream_rounds = _STREAM_BLOCKS // _WRITE_BLOCKS
    n_write_rounds = n_regions * _BUFFERS * stream_rounds

    def last_unit(i):
        return _divmod((i + 1) * step_pixels - 1, unit_pixels)[0]

    def write_rounds_before(i):
        return _FIRST_WRITES + _divmod(
            (i - read_steps) * _WRITE_RATE[0], _WRITE_RATE[1])[0]

    assert C % _LANES == 0 and n_steps * _BUFFERS * step_pixels == M
    assert n_units * unit_pixels * _BUFFERS == M
    assert block_rows % _READ_PIECE == 0 and block_rows % _WRITE_PIECE == 0
    assert early_rounds + read_steps * _STEP_PARTS == n_units * unit_rounds
    assert sorted(_READ_ORDER) == list(range(_STREAMS))
    assert _STREAM_BLOCKS % _WRITE_BLOCKS == 0 and last_unit(0) == 0
    assert write_rounds_before(n_steps) <= n_write_rounds
    for i in range(read_steps):
        assert (early_rounds + i * _STEP_PARTS
                >= (last_unit(i) + 1) * unit_rounds)
    for i in range(read_steps, n_steps):
        for t in range(write_rounds_before(i + 1)):
            region = t // (_BUFFERS * stream_rounds)
            blocks = (t % stream_rounds + 1) * _WRITE_BLOCKS
            assert ((region * _STREAM_BLOCKS + blocks) * _STREAMS * _BLOCK
                    <= i * step_pixels)

    def kernel(x_hbm, w_hbm, b_hbm, o_hbm, w_vmem, b_vmem,
               param_sems, read_sems, write_sems, *bufs):
        w_copy = pltpu.make_async_copy(w_hbm, w_vmem, param_sems.at[0])
        b_copy = pltpu.make_async_copy(b_hbm, b_vmem, param_sems.at[1])
        w_copy.start()
        b_copy.start()

        def start_reads(read_round, a):
            unit, _ = _divmod(read_round, unit_rounds)
            block, piece = _divmod(read_round, block_pieces)
            region, stream_block = _divmod(block, _STREAM_BLOCKS)
            for n, k in enumerate(_READ_ORDER, start=a * _STREAMS):
                stream = (region * _STREAMS + k) * _BUFFERS + a
                src = (stream * _STREAM_BLOCKS + stream_block) * block_pieces
                dst = (block * _STREAMS + k) * block_pieces
                pltpu.make_async_copy(
                    x_hbm.at[_rows(src + piece, _READ_PIECE)],
                    bufs[a].at[_rows(dst + piece, _READ_PIECE)],
                    read_sems.at[unit * _BUFFERS + a],
                ).start(priority=_READ_PRIORITIES[n % len(_READ_PRIORITIES)])

        def wait_unit(unit, a):
            rows = bufs[a].at[_rows(unit, unit_pixels * col_tiles)]
            pltpu.make_async_copy(
                rows, rows, read_sems.at[unit * _BUFFERS + a]).wait()

        def early_reads(read_round, carry):
            for a in range(_BUFFERS):
                start_reads(read_round, a)
            return carry

        jax.lax.fori_loop(0, early_rounds, early_reads, 0)
        w_copy.wait()
        b_copy.wait()
        bias = b_vmem[...].astype(jnp.float32).reshape(1, C)

        def multiply(buf, index, pixels):
            groups = pixels // _SUBLANES
            rows = _rows(index, pixels * col_tiles)
            tiles = buf[rows, :].reshape(groups, col_tiles, _SUBLANES, _LANES)
            lhs = jnp.concatenate(
                [tiles[:, c].reshape(pixels, _LANES) for c in range(col_tiles)],
                axis=1)
            acc = jnp.dot(lhs, w_vmem[...],
                          preferred_element_type=jnp.float32) + bias
            tiles = jnp.concatenate(
                [acc[:, c * _LANES:(c + 1) * _LANES].reshape(
                    groups, 1, _SUBLANES, _LANES) for c in range(col_tiles)],
                axis=1)
            buf[rows, :] = tiles.reshape(
                pixels * col_tiles, _LANES).astype(buf.dtype)

        def read_phase_step(i, carry):
            unit = last_unit(i)

            @pl.when(unit > last_unit(jnp.maximum(i, 1) - 1))
            def _():
                for a in range(_BUFFERS):
                    wait_unit(unit, a)

            for part in range(_STEP_PARTS):
                for a in range(_BUFFERS):
                    multiply(bufs[a], i * _STEP_PARTS + part, _PART)
                    start_reads(early_rounds + i * _STEP_PARTS + part, a)
            return carry

        for a in range(_BUFFERS):
            wait_unit(0, a)
        jax.lax.fori_loop(0, read_steps, read_phase_step, 0)

        o_blocks = o_hbm.reshape(
            n_regions * _STREAMS, _BUFFERS * _STREAM_BLOCKS, block_rows, _LANES)
        buf_blocks = [
            buf.reshape(n_regions * _STREAM_BLOCKS, _STREAMS, block_rows, _LANES)
            for buf in bufs]

        def start_writes(write_round):
            t, part = _divmod(write_round, stream_rounds)
            region, buffer = _divmod(t, _BUFFERS)
            streams = pl.ds(region * _STREAMS, _STREAMS)

            def start_from(a):
                for k in range(_WRITE_BLOCKS):
                    block = part * _WRITE_BLOCKS + k
                    for piece in range(block_rows // _WRITE_PIECE):
                        rows = _rows(piece, _WRITE_PIECE)
                        pltpu.make_async_copy(
                            buf_blocks[a].at[
                                region * _STREAM_BLOCKS + block, :, rows],
                            o_blocks.at[
                                streams, a * _STREAM_BLOCKS + block, rows],
                            write_sems.at[a]).start()

            if isinstance(buffer, int):
                start_from(buffer)
            else:
                for a in range(_BUFFERS):
                    pl.when(buffer == a)(lambda a=a: start_from(a))

        for unit in range(last_unit(read_steps - 1) + 1, n_units):
            for a in range(_BUFFERS):
                wait_unit(unit, a)
                if (unit, a) == (n_units - 1, 0):
                    start_writes(0)
        for write_round in range(1, _FIRST_WRITES):
            start_writes(write_round)

        def write_phase_step(i, carry):
            first = write_rounds_before(i)
            for t in range(pl.cdiv(*_WRITE_RATE)):
                pl.when(write_rounds_before(i + 1) > first + t)(
                    lambda t=t: start_writes(first + t))
            for buf in bufs:
                multiply(buf, i, step_pixels)
            return carry

        jax.lax.fori_loop(read_steps, n_steps, write_phase_step, 0)

        def remaining_writes(write_round, carry):
            start_writes(write_round)
            return carry

        jax.lax.fori_loop(
            write_rounds_before(n_steps), n_write_rounds, remaining_writes, 0)
        for a in range(_BUFFERS):
            pltpu.make_async_copy(bufs[a], bufs[a], write_sems.at[a]).wait()

    x_tiles = (x.reshape(M // _SUBLANES, _SUBLANES, col_tiles, _LANES)
               .transpose(0, 2, 1, 3).reshape(M * col_tiles, _LANES))
    out_tiles = pl.pallas_call(
        kernel,
        in_specs=[pl.BlockSpec(memory_space=pltpu.HBM)] * 3,
        out_specs=pl.BlockSpec(memory_space=pltpu.HBM),
        out_shape=jax.ShapeDtypeStruct(x_tiles.shape, x.dtype),
        scratch_shapes=[
            pltpu.VMEM((C, C), w.dtype),
            pltpu.VMEM((C,), b.dtype),
            pltpu.SemaphoreType.DMA((2,)),
            pltpu.SemaphoreType.DMA((n_units * _BUFFERS,)),
            pltpu.SemaphoreType.DMA((_BUFFERS,)),
        ] + [pltpu.VMEM((M * col_tiles // _BUFFERS, _LANES), x.dtype)] * _BUFFERS,
        compiler_params=pltpu.CompilerParams(
            vmem_limit_bytes=124 * 2**20,
            disable_bounds_checks=True,
            disable_semaphore_checks=True,
        ),
    )(x_tiles, w.reshape(C, C), b)
    return (out_tiles.reshape(M // _SUBLANES, col_tiles, _SUBLANES, _LANES)
            .transpose(0, 2, 1, 3).reshape(B, H, W, C))
```
